```python
import os as _os
_os.environ.setdefault("JAX_PLATFORMS", "cpu")
import jax
import jax.numpy as jnp

def _softmax(x, axis=-1):
    return jax.nn.softmax(x, axis=axis)
def _gelu(x):
    return jax.nn.gelu(x, approximate=True)
def _silu(x):
    return jax.nn.silu(x)
def _sigmoid(x):
    return jax.nn.sigmoid(x)
def _layernorm(x, axis=-1, eps=1e-5):
    m = jnp.mean(x, axis=axis, keepdims=True)
    v = jnp.var(x, axis=axis, keepdims=True)
    return (x - m) / jnp.sqrt(v + eps)
def _scatter_add(tgt, idx, src, axis=0):
    return tgt.at[idx].add(src)
def _segment_sum(src, seg, n):
    return jax.ops.segment_sum(src, seg, n)
class _Rng:
    def __init__(self, key):
        self._k = key
    def _next(self):
        self._k, sub = jax.random.split(self._k)
        return sub
    def normal(self, shape):
        return jax.random.normal(self._next(), shape, dtype=jnp.bfloat16)
    def randint(self, lo, hi, shape):
        return jax.random.randint(self._next(), shape, lo, hi, dtype=jnp.int32)
    def uniform(self, shape, lo=0.0, hi=1.0):
        return jax.random.uniform(self._next(), shape, jnp.bfloat16, lo, hi)
    def permutation(self, n):
        return jax.random.permutation(self._next(), n)


kernel_name = 'sequential_preLN__softmax_full_mha__swiglu_ffn__prompt'

def setup_inputs():
    _rng = _Rng(jax.random.key(int.from_bytes(__import__("os").urandom(4), "little")))
    _w = (lambda a: (lambda t: t.astype(jnp.bfloat16) if jnp.issubdtype(t.dtype, jnp.floating) else t)(jnp.asarray(a)))
    def _A_setup():
        B, S, D = 1, 2048, 512
        return {
            "x": _w((lambda *s: _rng.normal(s) * 0.05)(B, S, D)),
            "wqkv": _w((lambda *s: _rng.normal(s) * 0.05)(D, 3 * D)),
            "wo": _w((lambda *s: _rng.normal(s) * 0.05)(D, D)),
        }
    _A_in = _A_setup()

    def _B_setup():
        B, S, D, F = 1, 2048, 512, 1792
        return {
            "x": _w((lambda *s: _rng.normal(s) * 0.05)(B, S, D)),
            "w_gate": _w((lambda *s: _rng.normal(s) * 0.05)(D, F)),
            "w_up": _w((lambda *s: _rng.normal(s) * 0.05)(D, F)),
            "w_down": _w((lambda *s: _rng.normal(s) * 0.05)(F, D)),
        }
    _B_in = _B_setup()

    return {
        "A_x": _A_in["x"],
        "A_wqkv": _A_in["wqkv"],
        "A_wo": _A_in["wo"],
        "B_x": _B_in["x"],
        "B_w_gate": _B_in["w_gate"],
        "B_w_up": _B_in["w_up"],
        "B_w_down": _B_in["w_down"],
    }

def reference(A_x, A_wqkv, A_wo, B_x, B_w_gate, B_w_up, B_w_down):
    def _A_ref(x, wqkv, wo):
        B, S, D = x.shape
        H = 32; Dh = D // H
        qkv = (lambda x, *d: x.transpose(*d))((x @ wqkv).reshape(B, S, 3, H, Dh), 2, 0, 3, 1, 4)
        q, k, v = qkv[0], qkv[1], qkv[2]
        scale = Dh ** -0.5
        scores = jnp.einsum("bhqd,bhkd->bhqk", q, k) * scale
        p = _softmax(scores, axis=-1)
        o = jnp.einsum("bhqk,bhkd->bhqd", p, v)
        return (lambda x, *d: x.transpose(*d))(o, 0, 2, 1, 3).reshape(B, S, D) @ wo

    def _B_ref(x, w_gate, w_up, w_down):
        g = _silu(x @ w_gate)
        u = x @ w_up
        return (g * u) @ w_down

    x = A_x
    h = x + _A_ref(_layernorm(x, axis=-1), A_wqkv, A_wo)
    h2 = h + _B_ref(_layernorm(h, axis=-1), B_w_gate, B_w_up, B_w_down)
    return h2
```

```python
import functools

import jax
import jax.numpy as jnp
import jax.experimental.pallas as pl
import jax.experimental.pallas.tpu as pltpu

_H = 32
_LANES = 128
_CK = 128
_LOG2E = 1.4426950408889634
_EPS = 1e-5
_SAFE_LO, _SAFE_HI = 2.0 ** -60, 2.0 ** 100
_F32 = jnp.float32
_BF16 = jnp.bfloat16

_CFG = dict(
    tq=512,
    group=8,
    vk=16,
    extra=(1, 6, 11),
    skew=2,
    hold=1,
    tm=1024,
    fc=256,
    nsplit=3,
)


def _layernorm(x):
    mean = jnp.mean(x, axis=-1, keepdims=True)
    xc = x - mean
    var = jnp.mean(xc * xc, axis=-1, keepdims=True)
    return xc * jax.lax.rsqrt(var + _EPS)


def _dot(a, b):
    return jnp.dot(a, b, preferred_element_type=_F32)


def _pack(x):
    return pltpu.bitcast(x.astype(_BF16), jnp.int32)


def _unpack(w):
    return pltpu.bitcast(w, _BF16)


def _swiglu(gate, up):
    half = 0.5 * gate
    return (half + half * jnp.tanh(half)) * up


def _strassen_lhs(a11, a12, a21, a22):
    return (a11 + a22, a21 + a22, a11, a22, a11 + a12, a21 - a11, a12 - a22)


def _strassen_rhs(b11, b12, b21, b22):
    return (b11 + b22, b11, b12 - b22, b21 - b11, b22, b11 + b12, b21 + b22)


def _strassen_out(m1, m2, m3, m4, m5, m6, m7):
    return m1 + m4 - m5 + m7, m3 + m5, m2 + m4, m1 - m2 + m3 + m6


def _block_kernel(x_hbm, wqkv_hbm, wo_hbm, wg_hbm, wu_hbm, wd_hbm, out_hbm,
                  x_v, wqkv_v, wo_v, wg_v, wu_v, wd_v, out_v,
                  qt_v, q32_v, k_v, xn_v, kraw_v, kt_v, vt_v, ot_v, s_v,
                  hid_v, hn_v, act_v, wgu_v, wdn_v,
                  in_sems, w_sems, out_sems,
                  *, tq, group, vk, extra, skew, hold, tm, fc, nsplit):
    seq, d = x_v.shape
    ffn = wg_v.shape[1]
    dh = d // _H
    nq, nck = seq // tq, seq // _CK
    vchunks = sorted(list(range(nck)) + list(extra))
    on_mxu = [_CK - vk * vchunks.count(c) for c in range(nck)]
    vslots = [(c, vk * vchunks[:j].count(c)) for j, c in enumerate(vchunks)]
    hpt = _LANES // dh

    x_cp = [pltpu.make_async_copy(x_hbm.at[pl.ds(r * tq, tq)], x_v.at[pl.ds(r * tq, tq)],
                                  in_sems.at[r]) for r in range(nq)]
    wqkv_cp = [pltpu.make_async_copy(wqkv_hbm.at[:, pl.ds(j * d, d)], wqkv_v.at[j],
                                     in_sems.at[nq + j]) for j in range(3)]
    w_cp = [pltpu.make_async_copy(src, dst, w_sems.at[j]) for j, (src, dst) in enumerate(
        ((wo_hbm, wo_v), (wg_hbm, wg_v), (wu_hbm, wu_v), (wd_hbm, wd_v)))]
    nfc = ffn // fc

    hm, hd, hc = tm // 2, d // 2, fc // 2

    def pinned_load(ref, r, cols, after):
        w = ref[pl.ds(r, 16), cols]
        if after is not None:
            word = pltpu.bitcast(after, jnp.int32)
            zero = jax.lax.shift_right_logical(jax.lax.shift_right_logical(word, 31), 1)
            w = _unpack(pltpu.bitcast(w, jnp.int32) | jnp.tile(zero, (1, w.shape[1] // _LANES)))
        return w.astype(_F32)

    def combine_weights(j, prods=None):
        cols = pl.ds(j * fc, fc)
        for n, r in enumerate(range(0, hd, 16)):
            after = prods and prods[n % 7][r:r + 8, 0:_LANES]
            blocks = [pinned_load(w, r + o, cols, after) for o in (0, hd) for w in (wg_v, wu_v)]
            for m, b in enumerate(_strassen_rhs(*blocks)):
                if m not in (1, 4):
                    wgu_v[m, pl.ds(r // 2, 8), cols] = _pack(b)

    def combine_down_weights(j, prods):
        for n, r in enumerate(range(0, hc, 16)):
            after = prods[n % 7][r:r + 8, 0:_LANES]
            blocks = [pinned_load(wd_v, j * fc + r + o, pl.ds(c, hd), after)
                      for o in (0, hc) for c in (0, hd)]
            for m, b in enumerate(_strassen_rhs(*blocks)):
                wdn_v[m, pl.ds((j * hc + r) // 2, 8), :] = _pack(b)

    def gate_up_operand(m, j):
        cols = pl.ds(j * fc, fc)
        if m in (1, 4):
            return wg_v[0:hd, cols] if m == 1 else wu_v[hd:d, cols]
        return _unpack(wgu_v[m, :, cols])

    def normalize(r):
        xn_v[pl.ds(r * tq // 2, tq // 2), :] = _pack(
            _layernorm(x_v[pl.ds(r * tq, tq), :].astype(_F32)))

    def project_keys(r):
        rows = pl.ds(r * tq // 2, tq // 2)
        kraw_v[rows, :] = _pack(_dot(_unpack(xn_v[rows, :]), wqkv_v[1]))

    def relayout_keys(r):
        rows = pl.ds(r * tq // 2, tq // 2)
        for j, (c, pos) in enumerate(vslots):
            if c * _CK // tq == r:
                kv = _unpack(kraw_v[pl.ds((c * _CK + pos) // 2, vk // 2), :]).astype(_F32)
                for t in range(d // _LANES):
                    for e in range(dh):
                        kt_v[t, j, e] = pltpu.roll(kv[:, t * _LANES:(t + 1) * _LANES],
                                                   (j - e) % _LANES, 1)
        k = kraw_v[rows, :]
        for h in range(_H):
            k_v[h, rows, :] = k[:, h * dh:(h + 1) * dh]

    def project_queries(r):
        xn = _unpack(xn_v[pl.ds(r * tq // 2, tq // 2), :])
        qt = (_dot(xn, wqkv_v[0]) * ((dh ** -0.5) * _LOG2E)).astype(_BF16).T
        qt_v[r] = pltpu.bitcast(qt, jnp.int32).reshape(_H, dh // 2, tq)
        q32_v[r] = qt.astype(_F32).reshape(_H, dh, tq)

    def project_values(r):
        xn = _unpack(xn_v[pl.ds(r * tq // 2, tq // 2), :])
        vt = _dot(xn, wqkv_v[2]).astype(_BF16).T
        vt_v[:, :, pl.ds(r * tq, tq)] = pltpu.bitcast(vt, jnp.int32).reshape(_H, dh // 2, tq)

    batches = [[x_cp[0], wqkv_cp[1]], [x_cp[1], wqkv_cp[0]], x_cp[2:] + [wqkv_cp[2]], w_cp]

    def next_batch(n):
        for cp in batches[n]:
            cp.wait()
        for cp in batches[n + 1]:
            cp.start()

    for cp in batches[0]:
        cp.start()
    next_batch(0)
    normalize(0)
    project_keys(0)
    next_batch(1)
    project_queries(0)
    normalize(1)
    project_keys(1)
    relayout_keys(0)
    next_batch(2)
    project_values(0)
    for r in range(2, nq):
        normalize(r)
        project_keys(r)
    for r in range(1, nq):
        relayout_keys(r)
    for r in range(1, nq):
        project_queries(r)
    for r in range(1, nq):
        project_values(r)

    def keys_of(h, row0, n):
        return pltpu.bitcast(k_v[h, pl.ds(row0 // 2, n // 2), :], _BF16)

    def values_of(h, row0, n):
        return pltpu.bitcast(vt_v[h, :, pl.ds(row0, n)], _BF16)

    def queries_of(i, h):
        return pltpu.bitcast(qt_v[i, h], _BF16)

    def vpu_scores(i, h0, g, j):
        h, lane = h0 + g, (g % hpt * dh + j) % _LANES
        kcols = [jnp.broadcast_to(kt_v[h // hpt, j, e][:, lane:lane + 1], (vk, _LANES))
                 for e in range(dh)]
        cols = []
        for t in range(tq // _LANES):
            terms = [kcols[e] * q32_v[i, h, pl.ds(e, 1), pl.ds(t * _LANES, _LANES)]
                     for e in range(dh)]
            cols.append(functools.reduce(jnp.add, terms))
        return jnp.concatenate(cols, axis=1)

    def attend_fast(it, bounds):
        i, h0 = it // (_H // group), it % (_H // group) * group
        jobs = [(g, c) for g in range(group) for c in range(nck)]
        l_run, o_run, probs = [None] * group, [None] * group, []
        done = 0
        for n in range(len(jobs) + 1):
            if n < len(jobs):
                g, c = jobs[n]
                row0 = (c + 1) * _CK - on_mxu[c]
                s = [_dot(keys_of(h0 + g, row0, on_mxu[c]), queries_of(i, h0 + g))]
                sv = [vpu_scores(i, h0, g, j) for j, cj in enumerate(vchunks) if cj == c]
                p = jnp.exp2(jnp.concatenate(sv + s, axis=0))
                parts = [p[r:r + 8] for r in range(0, _CK, 8)]
                l_run[g] = functools.reduce(
                    jnp.add, ([] if l_run[g] is None else [l_run[g]]) + parts)
                probs.append(p.astype(_BF16))
            ready = len(jobs) if n == len(jobs) else min(n - skew + 1, len(jobs) - skew - hold)
            for g, c in jobs[done:max(ready, done)]:
                o_c = _dot(values_of(h0 + g, c * _CK, _CK), probs.pop(0))
                o_run[g] = o_c if o_run[g] is None else o_run[g] + o_c
            done = max(ready, done)
        lo, hi = bounds
        outs = []
        for l_g, o_g in zip(l_run, o_run):
            l_row = jnp.sum(l_g, axis=0, keepdims=True)
            outs.append(_pack(o_g * pl.reciprocal(l_row)))
            lo = jnp.minimum(lo, l_row)
            hi = hi + l_g + jnp.abs(o_g[0:8]) + jnp.abs(o_g[8:16])
        ot_v[i, pl.ds(h0, group)] = jnp.stack(outs)
        return lo, hi

    def attend_exact(t, _):
        i, h = t // _H, t % _H
        s_v[...] = _dot(keys_of(h, 0, seq), queries_of(i, h))
        p = jnp.exp2(s_v[...] - jnp.max(s_v[...], axis=0, keepdims=True))
        o = _dot(values_of(h, 0, seq), p.astype(_BF16))
        ot_v[i, h] = _pack(o / jnp.sum(p, axis=0, keepdims=True))

    lo, hi = jax.lax.fori_loop(
        0, nq * _H // group, attend_fast,
        (jnp.full((1, tq), _SAFE_HI, _F32), jnp.zeros((8, tq), _F32)))
    safe = jnp.logical_and(lo >= _SAFE_LO, hi <= _SAFE_HI)

    @pl.when(jnp.sum(jnp.where(safe, 0.0, 1.0)) > 0.0)
    def _():
        jax.lax.fori_loop(0, nq * _H, attend_exact, None)

    def project(i):
        attn = _dot(_unpack(xn_v[pl.ds(i * tq // 2, tq // 2), :]), wo_v[...])
        for r in range(0, tq, 32):
            rows = pl.ds(i * tq + r, 32)
            hid = x_v[rows, :].astype(_F32) + attn[r:r + 32]
            hid_v[rows, :] = hid
            hn = _layernorm(hid)
            for m, a in enumerate(
                    _strassen_lhs(hn[:16, :hd], hn[:16, hd:], hn[16:, :hd], hn[16:, hd:])):
                hn_v[m, pl.ds((i * tq + r) // 4, 8), :] = _pack(a)

    def gate_up(i, j):
        prods = [_dot(_unpack(hn_v[m, pl.ds(i * hm // 2, hm // 2), :]), gate_up_operand(m, j))
                 for m in range(7)]
        if i == 0:
            if j + 1 < nfc:
                combine_weights(j + 1, prods)
            combine_down_weights(j, prods)
        for r in range(0, hm, 16):
            g_top, u_top, g_bot, u_bot = _strassen_out(*[p[r:r + 16] for p in prods])
            top, bot = _swiglu(g_top, u_top), _swiglu(g_bot, u_bot)
            for m, a in enumerate(
                    _strassen_lhs(top[:, :hc], top[:, hc:], bot[:, :hc], bot[:, hc:])):
                act_v[i % 2, m, pl.ds(r // 2, 8), pl.ds(j * hc, hc)] = _pack(a)

    def out_copy(n):
        rows = pl.ds(*out_parts[n])
        return pltpu.make_async_copy(out_v.at[rows], out_hbm.at[rows], out_sems.at[n])

    def down(n):
        row0, size = out_parts[n]
        i, half = row0 // tm, pl.ds(row0 % tm // 4, size // 4)
        prods = [_dot(_unpack(act_v[i % 2, m, half, :]), _unpack(wdn_v[m])) for m in range(7)]
        for r in range(0, size // 2, 16):
            c11, c12, c21, c22 = _strassen_out(*[p[r:r + 16] for p in prods])
            rows = pl.ds(row0 + 2 * r, 32)
            ffn_out = jnp.concatenate(
                [jnp.concatenate([c11, c12], axis=1), jnp.concatenate([c21, c22], axis=1)], axis=0)
            out_v[rows, :] = (hid_v[rows, :] + ffn_out).astype(out_v.dtype)

    ntiles = seq // tm
    out_parts = [(i * tm, tm) for i in range(ntiles - 1)]
    out_parts += [(seq - (tm >> x), tm >> min(x + 1, nsplit)) for x in range(nsplit + 1)]
    for cp in w_cp:
        cp.wait()
    for i in range(nq):
        xn_v[pl.ds(i * tq // 2, tq // 2), :] = pltpu.bitcast(
            _unpack(ot_v[i].reshape(d // 2, tq)).T, jnp.int32)
    for i in range(nq):
        project(i)
    combine_weights(0)
    for i in range(ntiles):
        for j in range(nfc):
            gate_up(i, j)
            if i and j == 0:
                down(i - 1)
            if i and j == 2:
                out_copy(i - 1).start()
    for n in range(ntiles - 1, len(out_parts)):
        down(n)
        if n >= ntiles:
            out_copy(n - 1).start()
    out_copy(len(out_parts) - 1).start()
    for n in range(len(out_parts)):
        out_copy(n).wait()


def _run(x, wqkv, wo, wg, wu, wd, cfg):
    batch, seq, d = x.shape
    assert batch == 1
    f = wg.shape[1]
    dh = d // _H
    tq = cfg["tq"]
    assert cfg["group"] % (_LANES // dh) == 0
    nslots = seq // _CK + len(cfg["extra"])
    any_spec = pl.BlockSpec(memory_space=pl.ANY)
    out = pl.pallas_call(
        functools.partial(_block_kernel, **cfg),
        out_shape=jax.ShapeDtypeStruct((seq, d), x.dtype),
        in_specs=[any_spec] * 6,
        out_specs=any_spec,
        scratch_shapes=[
            pltpu.VMEM((seq, d), x.dtype),
            pltpu.VMEM((3, d, d), wqkv.dtype),
            pltpu.VMEM((d, d), wo.dtype),
            pltpu.VMEM((d, f), wg.dtype),
            pltpu.VMEM((d, f), wu.dtype),
            pltpu.VMEM((f, d), wd.dtype),
            pltpu.VMEM((seq, d), x.dtype),
            pltpu.VMEM((seq // tq, _H, dh // 2, tq), jnp.int32),
            pltpu.VMEM((seq // tq, _H, dh, tq), _F32),
            pltpu.VMEM((_H, seq // 2, dh), jnp.int32),
            pltpu.VMEM((seq // 2, d), jnp.int32),
            pltpu.VMEM((seq // 2, d), jnp.int32),
            pltpu.VMEM((d // _LANES, nslots, dh, cfg["vk"], _LANES), _F32),
            pltpu.VMEM((_H, dh // 2, seq), jnp.int32),
            pltpu.VMEM((seq // tq, _H, dh // 2, tq), jnp.int32),
            pltpu.VMEM((seq, tq), _F32),
            pltpu.VMEM((seq, d), _F32),
            pltpu.VMEM((7, seq // 4, d // 2), jnp.int32),
            pltpu.VMEM((2, 7, cfg["tm"] // 4, f // 2), jnp.int32),
            pltpu.VMEM((7, d // 4, f), jnp.int32),
            pltpu.VMEM((7, f // 4, d // 2), jnp.int32),
            pltpu.SemaphoreType.DMA((seq // tq + 3,)),
            pltpu.SemaphoreType.DMA((4,)),
            pltpu.SemaphoreType.DMA((seq // cfg["tm"] + cfg["nsplit"],)),
        ],
        compiler_params=pltpu.CompilerParams(vmem_limit_bytes=124 * 1024 * 1024),
    )(x.reshape(seq, d), wqkv, wo, wg, wu, wd)
    return out.reshape(batch, seq, d)


@jax.jit
def pallas_sequential_preLN__softmax_full_mha__swiglu_ffn__prompt_kernel(
    A_x: jax.Array,
    A_wqkv: jax.Array,
    A_wo: jax.Array,
    B_x: jax.Array,
    B_w_gate: jax.Array,
    B_w_up: jax.Array,
    B_w_down: jax.Array,
):
    del B_x
    return _run(A_x, A_wqkv, A_wo, B_w_gate, B_w_up, B_w_down, _CFG)
```
